```python
import os as _os
_os.environ.setdefault("JAX_PLATFORMS", "cpu")
import jax
import jax.numpy as jnp

def _softmax(x, axis=-1):
    return jax.nn.softmax(x, axis=axis)
def _gelu(x):
    return jax.nn.gelu(x, approximate=True)
def _silu(x):
    return jax.nn.silu(x)
def _sigmoid(x):
    return jax.nn.sigmoid(x)
def _layernorm(x, axis=-1, eps=1e-5):
    m = jnp.mean(x, axis=axis, keepdims=True)
    v = jnp.var(x, axis=axis, keepdims=True)
    return (x - m) / jnp.sqrt(v + eps)
def _scatter_add(tgt, idx, src, axis=0):
    return tgt.at[idx].add(src)
def _segment_sum(src, seg, n):
    return jax.ops.segment_sum(src, seg, n)
class _Rng:
    def __init__(self, key):
        self._k = key
    def _next(self):
        self._k, sub = jax.random.split(self._k)
        return sub
    def normal(self, shape):
        return jax.random.normal(self._next(), shape, dtype=jnp.bfloat16)
    def randint(self, lo, hi, shape):
        return jax.random.randint(self._next(), shape, lo, hi, dtype=jnp.int32)
    def uniform(self, shape, lo=0.0, hi=1.0):
        return jax.random.uniform(self._next(), shape, jnp.bfloat16, lo, hi)
    def permutation(self, n):
        return jax.random.permutation(self._next(), n)


kernel_name = 'concat_heads__sliding_block_cached__mha_block_cached__decode'

def setup_inputs():
    _rng = _Rng(jax.random.key(int.from_bytes(__import__("os").urandom(4), "little")))
    _w = (lambda a: (lambda t: t.astype(jnp.bfloat16) if jnp.issubdtype(t.dtype, jnp.floating) else t)(jnp.asarray(a)))
    def _A_setup():
        B, Sq, D = 4, 1, 640
        Hq, Hkv, Sk, Dh = 32, 32, 4096, 128
        assert Hq % Hkv == 0, (Hq, Hkv)
        return {
            "x": _w((lambda *s: _rng.normal(s) * 0.8)(B, Sq, D)),
            "k_cache": _w((lambda *s: _rng.normal(s) * 0.8)(B, Hkv, Sk, Dh)),
            "v_cache": _w((lambda *s: _rng.normal(s) * 0.05)(B, Hkv, Sk, Dh)),
            "wq": _w((lambda *s: _rng.normal(s) * 0.8)(D, Hq * Dh) * (D ** -0.5)),
            "wo": _w((lambda *s: _rng.normal(s) * 0.05)(Hq * Dh, D) * ((Hq * Dh) ** -0.5)),
        }
    _A_in = _A_setup()

    def _B_setup():
        B, Sq, D = 4, 1, 640
        H, Sk, Dh = 32, 4096, 128
        return {
            "x": _w((lambda *s: _rng.normal(s) * 0.8)(B, Sq, D)),
            "k_cache": _w((lambda *s: _rng.normal(s) * 0.8)(B, H, Sk, Dh)),
            "v_cache": _w((lambda *s: _rng.normal(s) * 0.05)(B, H, Sk, Dh)),
            "wq": _w((lambda *s: _rng.normal(s) * 0.8)(D, H * Dh) * (D ** -0.5)),
            "wo": _w((lambda *s: _rng.normal(s) * 0.05)(H * Dh, D) * ((H * Dh) ** -0.5)),
        }
    _B_in = _B_setup()

    return {
        "A_x": _A_in["x"],
        "A_k_cache": _A_in["k_cache"],
        "A_v_cache": _A_in["v_cache"],
        "A_wq": _A_in["wq"],
        "A_wo": _A_in["wo"],
        "B_x": _B_in["x"],
        "B_k_cache": _B_in["k_cache"],
        "B_v_cache": _B_in["v_cache"],
        "B_wq": _B_in["wq"],
        "B_wo": _B_in["wo"],
    }

def reference(A_x, A_k_cache, A_v_cache, A_wq, A_wo, B_x, B_k_cache, B_v_cache, B_wq, B_wo):
    def _A_ref(x, k_cache, v_cache, wq, wo):
        B, Sq, D = x.shape
        Hq, Dh = 32, 128
        Hkv, Sk = k_cache.shape[1], k_cache.shape[2]
        W = min(4096, max(256, Sk // 4))
        rep = Hq // Hkv
        q = (lambda x, *d: x.transpose(*d))((x @ wq).reshape(B, Sq, Hq, Dh), 0, 2, 1, 3)
        k = jnp.repeat(k_cache[:, :, Sk - W:, :], rep, axis=1)
        v = jnp.repeat(v_cache[:, :, Sk - W:, :], rep, axis=1)
        scores = jnp.einsum("bhqd,bhkd->bhqk", q, k) * (Dh ** -0.5)
        p = _softmax(scores, axis=-1)
        o = jnp.einsum("bhqk,bhkd->bhqd", p, v)
        return (lambda x, *d: x.transpose(*d))(o, 0, 2, 1, 3).reshape(B, Sq, Hq * Dh) @ wo

    def _B_ref(x, k_cache, v_cache, wq, wo):
        B, Sq, D = x.shape
        H, Dh = 32, 128
        q = (lambda x, *d: x.transpose(*d))((x @ wq).reshape(B, Sq, H, Dh), 0, 2, 1, 3)
        scores = jnp.einsum("bhqd,bhkd->bhqk", q, k_cache) * (Dh ** -0.5)
        p = _softmax(scores, axis=-1)
        o = jnp.einsum("bhqk,bhkd->bhqd", p, v_cache)
        return (lambda x, *d: x.transpose(*d))(o, 0, 2, 1, 3).reshape(B, Sq, H * Dh) @ wo

    a = _A_ref(A_x, A_k_cache, A_v_cache, A_wq, A_wo)
    b = _B_ref(B_x, B_k_cache, B_v_cache, B_wq, B_wo)
    return jnp.concatenate([a, b], axis=-1)
```

```python
import functools
import jax
import jax.numpy as jnp
from jax import lax
import jax.experimental.pallas as pl
import jax.experimental.pallas.tpu as pltpu

NT = (((1,), (1,)), ((), ()))
HG = 8
SB = 512
CR = 16
NBUF = 3
NWQ = 4
NWO = 4


def _kernel(ax_hbm, bx_hbm, awq_hbm, bwq_hbm, awo_hbm, bwo_hbm,
            ak_hbm, av_hbm, bk_hbm, bv_hbm, o_ref,
            x_buf, wq_buf, wo_buf, k_buf, v_buf, q_scr, o_scr,
            x_sem, wq_sem, wo_sem, kv_sem, *, scale, B, H, S, W, D, Dh):
    G = B * H // HG
    ncA, ncB = W // SB, S // SB
    nA, nB = G * ncA, G * ncB
    n = nA + nB
    HD = H * Dh
    wq_cols = HD // NWQ
    wo_rows = HD // NWO
    RG = wq_buf.shape[2]

    def issue_wq(c):
        for cc in range(wq_cols // 256):
            c0 = c * wq_cols + cc * 256
            for r0 in range(0, RG, 8):
                for a, src in enumerate((awq_hbm, bwq_hbm)):
                    pltpu.make_async_copy(
                        src.at[:, pl.ds(r0, 8), pl.ds(c0, 256)],
                        wq_buf.at[a, :, pl.ds(r0, 8), pl.ds(c0, 256)],
                        wq_sem.at[c, a]).start(priority=a)

    def wait_wq(c, a):
        dst = wq_buf.at[a, :, :, pl.ds(c * wq_cols, wq_cols)]
        pltpu.make_async_copy(dst, dst, wq_sem.at[c, a]).wait()

    def issue_wo(c):
        for r0 in range(c * wo_rows, (c + 1) * wo_rows, 16):
            for a, src in enumerate((awo_hbm, bwo_hbm)):
                pltpu.make_async_copy(
                    src.at[pl.ds(r0, 16)], wo_buf.at[a, pl.ds(r0, 16)],
                    wo_sem.at[c, a]).start(priority=a)

    def wait_wo(c, a):
        dst = wo_buf.at[a, pl.ds(c * wo_rows, wo_rows)]
        pltpu.make_async_copy(dst, dst, wo_sem.at[c, a]).wait()

    def issue_kv(k_hbm, v_hbm, g, s0, slot):
        h0 = g * HG
        for j in range(SB // CR):
            for a, (src, buf) in enumerate(((k_hbm, k_buf), (v_hbm, v_buf))):
                pltpu.make_async_copy(
                    src.at[pl.ds(h0, HG), pl.ds(s0 + j * CR, CR)],
                    buf.at[slot, :, pl.ds(j * CR, CR)],
                    kv_sem.at[slot, a]).start(priority=a)

    def issue_A(t, slot):
        issue_kv(ak_hbm, av_hbm, t // ncA, (S - W) + (t % ncA) * SB, slot)

    def issue_B(t, slot):
        tb = t - nA
        issue_kv(bk_hbm, bv_hbm, tb // ncB, (tb % ncB) * SB, slot)

    def wait_kv(slot, a):
        buf = (k_buf, v_buf)[a]
        pltpu.make_async_copy(buf.at[slot], buf.at[slot], kv_sem.at[slot, a]).wait()

    def q_proj(c):
        for a in range(2):
            wait_wq(c, a)
            w = wq_buf[a, :, :, pl.ds(c * wq_cols, wq_cols)].reshape(D, wq_cols)
            q = jnp.dot(x_buf[a], w, preferred_element_type=jnp.float32)
            for j in range(wq_cols // Dh):
                h = c * (wq_cols // Dh) + j
                q_scr[a, pl.ds(h, B, stride=H), :] = q[:, j * Dh:(j + 1) * Dh]

    xa = pltpu.make_async_copy(ax_hbm, x_buf.at[0], x_sem.at[0])
    xb = pltpu.make_async_copy(bx_hbm, x_buf.at[1], x_sem.at[1])
    xa.start(); xb.start()
    issue_wq(0)
    issue_wq(1)
    xa.wait(); xb.wait()
    issue_wq(2)
    q_proj(0)
    issue_wq(3)
    q_proj(1)
    issue_A(0, 0)
    q_proj(2)
    issue_A(1, 1)
    q_proj(3)

    row = lax.broadcasted_iota(jnp.int32, (HG, SB), 0)
    row_o = lax.broadcasted_iota(jnp.int32, (HG, Dh), 0)

    def body(t, carry):
        m_old, l_old, acc_old = carry
        slot = lax.rem(t, NBUF)
        t2 = t + 2
        slot2 = lax.rem(t2, NBUF)

        @pl.when(t2 < nA)
        def _():
            issue_A(t2, slot2)

        @pl.when(jnp.logical_and(t2 >= nA, t2 < n))
        def _():
            issue_B(t2, slot2)

        @pl.when(t2 == n)
        def _():
            issue_wo(0)

        @pl.when(t2 == n + 1)
        def _():
            issue_wo(1)

        is_a = t < nA
        tb = t - nA
        br = jnp.where(is_a, 0, 1)
        g = jnp.where(is_a, t // ncA, tb // ncB)
        c = jnp.where(is_a, t % ncA, tb % ncB)
        last = jnp.where(is_a, ncA - 1, ncB - 1)
        first = c == 0
        grow = pl.multiple_of(g * HG, HG)

        q8 = q_scr[br, pl.ds(grow, HG), :].astype(jnp.bfloat16)
        wait_kv(slot, 0)
        s = None
        for j in range(HG):
            sj = lax.dot_general(q8, k_buf[slot, j], NT, preferred_element_type=jnp.float32)
            s = sj if s is None else jnp.where(row == j, sj, s)
        s = s * scale
        m_old = jnp.where(first, -jnp.inf, m_old)
        l_old = jnp.where(first, 0.0, l_old)
        acc_old = jnp.where(first, 0.0, acc_old)
        m_new = jnp.maximum(m_old, jnp.max(s, axis=-1, keepdims=True))
        alpha = jnp.exp(m_old - m_new)
        p = jnp.exp(s - m_new[:, 0:1])
        psum = p[:, 0:Dh]
        for i in range(1, SB // Dh):
            psum = psum + p[:, i * Dh:(i + 1) * Dh]
        l_new = alpha * l_old + psum
        pb = p.astype(jnp.bfloat16)
        wait_kv(slot, 1)
        pv = None
        for j in range(HG):
            oj = jnp.dot(pb, v_buf[slot, j], preferred_element_type=jnp.float32)
            pv = oj if pv is None else jnp.where(row_o == j, oj, pv)
        acc_new = alpha * acc_old + pv

        @pl.when(c == last)
        def _():
            o_scr[br, pl.ds(grow, HG), :] = acc_new / jnp.sum(l_new, axis=-1, keepdims=True)

        return m_new, l_new, acc_new

    z = jnp.zeros((HG, Dh), jnp.float32)
    lax.fori_loop(0, n, body, (z, z, z))

    y = [None, None]
    for c in range(NWO):
        if c + 2 < NWO:
            issue_wo(c + 2)
        for a in range(2):
            lhs = jnp.concatenate(
                [o_scr[a, pl.ds(c * (wo_rows // Dh) + j, B, stride=H), :] for j in range(wo_rows // Dh)],
                axis=-1).astype(jnp.bfloat16)
            wait_wo(c, a)
            part = jnp.dot(lhs, wo_buf[a, pl.ds(c * wo_rows, wo_rows), :], preferred_element_type=jnp.float32)
            y[a] = part if y[a] is None else y[a] + part
    o_ref[:, 0:D] = y[0].astype(o_ref.dtype)
    o_ref[:, D:2 * D] = y[1].astype(o_ref.dtype)


@jax.jit
def pallas_concat_heads__sliding_block_cached__mha_block_cached__decode_kernel(
    A_x, A_k_cache, A_v_cache, A_wq, A_wo, B_x, B_k_cache, B_v_cache, B_wq, B_wo):
    B, Sq, D = A_x.shape
    _, H, S, Dh = A_k_cache.shape
    W = min(4096, max(256, S // 4))
    scale = Dh ** -0.5
    HD = H * Dh
    any_spec = pl.BlockSpec(memory_space=pl.ANY)
    kv = lambda t: t.reshape(B * H, S, Dh)
    wq = lambda t: t.reshape(8, D // 8, HD)
    out = pl.pallas_call(
        functools.partial(_kernel, scale=scale, B=B, H=H, S=S, W=W, D=D, Dh=Dh),
        in_specs=[any_spec] * 10,
        out_specs=pl.BlockSpec(memory_space=pltpu.VMEM),
        out_shape=jax.ShapeDtypeStruct((B, 2 * D), A_x.dtype),
        scratch_shapes=[
            pltpu.VMEM((2, B, D), jnp.bfloat16),
            pltpu.VMEM((2, 8, D // 8, HD), jnp.bfloat16),
            pltpu.VMEM((2, HD, D), jnp.bfloat16),
            pltpu.VMEM((NBUF, HG, SB, Dh), jnp.bfloat16),
            pltpu.VMEM((NBUF, HG, SB, Dh), jnp.bfloat16),
            pltpu.VMEM((2, B * H, Dh), jnp.float32),
            pltpu.VMEM((2, B * H, Dh), jnp.float32),
            pltpu.SemaphoreType.DMA((2,)),
            pltpu.SemaphoreType.DMA((NWQ, 2)),
            pltpu.SemaphoreType.DMA((NWO, 2)),
            pltpu.SemaphoreType.DMA((NBUF, 2)),
        ],
        compiler_params=pltpu.CompilerParams(vmem_limit_bytes=64 * 1024 * 1024),
    )(A_x.reshape(B, D), B_x.reshape(B, D), wq(A_wq), wq(B_wq), A_wo, B_wo,
      kv(A_k_cache), kv(A_v_cache), kv(B_k_cache), kv(B_v_cache))
    return out.reshape(B, Sq, 2 * D)
```

```python
import functools
import jax
import jax.numpy as jnp
from jax import lax
import jax.experimental.pallas as pl
import jax.experimental.pallas.tpu as pltpu

NT = (((1,), (1,)), ((), ()))
HG = 8

DEFAULT = dict(SB=512, CR=16, NBUF=3, compute=True, kprio=0, wqprio=0, woprio=0, dbc=False,
               a_first=True, hoffA=2, hoffB=4, wq_cw=256, tail=4, qcols=1024, lead=1)
WQG = 5
WOG = 4


def _kernel(*refs, cfg, **kw):
    nsem = 2 + 2 + 2 * cfg['NBUF'] + 2 * (8 - 1 + cfg['tail'])
    pl.run_scoped(lambda sems: _kernel_inner(*refs, sems, cfg=cfg, **kw), pltpu.SemaphoreType.DMA((nsem,)))


def _kernel_inner(ax_hbm, bx_hbm, awq_hbm, bwq_hbm, awo_hbm, bwo_hbm,
                  ak_hbm, av_hbm, bk_hbm, bv_hbm, o_ref,
                  x_buf, wq_buf, wo_buf, k_buf, v_buf, q_scr, o_scr,
                  sems, *, scale, B, H, S, W, D, Dh, cfg):
    SB, CR, NBUF = cfg['SB'], cfg['CR'], cfg['NBUF']
    compute = cfg['compute']
    NH = B * H
    G = NH // HG
    ncA, ncB = W // SB, S // SB
    nA, nB = G * ncA, G * ncB
    n = nA + nB
    HD = H * Dh
    kp = cfg['kprio']
    TAIL = cfg['tail']
    hoffs = (cfg['hoffA'], cfg['hoffB'])
    x_sem = lambda a: sems.at[a]
    wq_sem = lambda a: sems.at[2 + a]
    kv_sem = lambda slot, a: sems.at[4 + 2 * slot + a]
    wo_sem = lambda i, a: sems.at[4 + 2 * NBUF + 2 * i + a]

    def issue_wq():
        CW = cfg['wq_cw']
        for r0 in range(0, wq_buf.shape[2], 8):
            for c0 in range(0, HD, CW):
                for a, src in enumerate((awq_hbm, bwq_hbm)):
                    pltpu.make_async_copy(
                        src.at[:, pl.ds(r0, 8), pl.ds(c0, CW)],
                        wq_buf.at[a, :, pl.ds(r0, 8), pl.ds(c0, CW)],
                        wq_sem(a)).start(priority=a ^ cfg['wqprio'])

    def wait_wq(a):
        pltpu.make_async_copy(wq_buf.at[a], wq_buf.at[a], wq_sem(a)).wait()

    NWO = wo_buf.shape[2] // Dh
    def wo_parts(c, a):
        if c < NWO - 1 or (a ^ cfg['woprio']) == 0:
            return [(0, WOG, c)]
        gw = WOG // TAIL
        return [(i * gw, gw, NWO - 1 + i) for i in range(TAIL)]

    def issue_wo(c):
        lists = []
        for a, src in enumerate((awo_hbm, bwo_hbm)):
            lst = []
            for (g0, gw, si) in wo_parts(c, a):
                pr = 8 * (WOG // gw)
                for r0 in range(c * Dh, (c + 1) * Dh, pr):
                    lst.append(pltpu.make_async_copy(
                        src.at[pl.ds(g0, gw), pl.ds(r0, pr)], wo_buf.at[a, pl.ds(g0, gw), pl.ds(r0, pr)],
                        wo_sem(si, a)))
            lists.append(lst)
        for da, db in zip(*lists):
            da.start(priority=cfg['woprio'])
            db.start(priority=1 ^ cfg['woprio'])

    def wait_wo(c, part, a):
        g0, gw, si = part
        dst = wo_buf.at[a, pl.ds(g0, gw), pl.ds(c * Dh, Dh)]
        pltpu.make_async_copy(dst, dst, wo_sem(si, a)).wait()

    def issue_kv_parts(k_hbm, v_hbm, parts, s0, slot):
        for j in range(SB // CR):
            for a, src, buf in ((0, k_hbm, k_buf), (1, v_hbm, v_buf)):
                for (h0, hn, d0) in parts:
                    pltpu.make_async_copy(
                        src.at[pl.ds(h0, hn), pl.ds(s0 + j * CR, CR)],
                        buf.at[slot, pl.ds(d0, hn), pl.ds(j * CR, CR)],
                        kv_sem(slot, a)).start(priority=a ^ kp)

    def issue_kv(k_hbm, v_hbm, g, s0, slot, hoff):
        plain = lambda: issue_kv_parts(k_hbm, v_hbm, [(g * HG + hoff, HG, 0)], s0, slot)
        wrap = lambda: issue_kv_parts(k_hbm, v_hbm, [(NH - (HG - hoff), HG - hoff, 0), (0, hoff, HG - hoff)], s0, slot)
        if hoff == 0:
            plain()
        elif isinstance(g, int):
            wrap() if g == G - 1 else plain()
        else:
            pl.when(g < G - 1)(plain)
            pl.when(g == G - 1)(wrap)

    a_first = cfg['a_first']
    offA = 0 if a_first else nB
    offB = nA if a_first else 0
    def issue_A(t, slot):
        ta = t - offA
        issue_kv(ak_hbm, av_hbm, ta // ncA, (S - W) + (ta % ncA) * SB, slot, hoffs[0])

    def issue_B(t, slot):
        tb = t - offB
        issue_kv(bk_hbm, bv_hbm, tb // ncB, (tb % ncB) * SB, slot, hoffs[1])

    issue_first = issue_A if a_first else issue_B

    def wait_kv(slot, a):
        buf = (k_buf, v_buf)[a]
        pltpu.make_async_copy(buf.at[slot], buf.at[slot], kv_sem(slot, a)).wait()

    def q_proj(a):
        wait_wq(a)
        if not compute: return
        QC = cfg['qcols']
        for c in range(HD // QC):
            w = wq_buf[a, :, :, pl.ds(c * QC, QC)].reshape(D, QC)
            q = jnp.dot(x_buf[a], w, preferred_element_type=jnp.float32)
            for j in range(QC // Dh):
                h = c * (QC // Dh) + j
                q_scr[a, pl.ds(h + HG - hoffs[a], B, stride=H), :] = q[:, j * Dh:(j + 1) * Dh]
                if h < hoffs[a]:
                    q_scr[a, pl.ds(NH + h + HG - hoffs[a], 1), :] = q[0:1, j * Dh:(j + 1) * Dh]

    xa = pltpu.make_async_copy(ax_hbm, x_buf.at[0], x_sem(0))
    xb = pltpu.make_async_copy(bx_hbm, x_buf.at[1], x_sem(1))
    xa.start(); xb.start(priority=1)
    issue_wq()
    for t in range(NBUF - 1):
        issue_first(t, t)
    xa.wait(); xb.wait()
    q_proj(0)
    issue_first(NBUF - 1, NBUF - 1)
    q_proj(1)

    row = lax.broadcasted_iota(jnp.int32, (HG, SB), 0)
    row_o = lax.broadcasted_iota(jnp.int32, (HG, Dh), 0)
    wo_per = 2

    def body(t, carry):
        m_old, l_old, acc_old = carry
        slot = lax.rem(t, NBUF)
        if compute:
            is_a = jnp.logical_and(t >= offA, t < offA + nA)
            ta = t - offA
            tb = t - offB
            br = jnp.where(is_a, 0, 1)
            g = jnp.where(is_a, ta // ncA, tb // ncB)
            c = jnp.where(is_a, ta % ncA, tb % ncB)
            last = jnp.where(is_a, ncA - 1, ncB - 1)
            first = c == 0
            grow = pl.multiple_of((g + 1) * HG, HG)

            q8 = q_scr[br, pl.ds(grow, HG), :].astype(jnp.bfloat16)
            wait_kv(slot, 0)
            s = None
            for j in range(HG):
                sj = lax.dot_general(q8, k_buf[slot, j], NT, preferred_element_type=jnp.float32)
                s = sj if s is None else jnp.where(row == j, sj, s)
            s = s * scale
            m_old = jnp.where(first, -jnp.inf, m_old)
            l_old = jnp.where(first, 0.0, l_old)
            acc_old = jnp.where(first, 0.0, acc_old)
            m_new = jnp.maximum(m_old, jnp.max(s, axis=-1, keepdims=True))
            alpha = jnp.exp(m_old - m_new)
            p = jnp.exp(s - m_new[:, 0:1])
            psum = p[:, 0:Dh]
            for i in range(1, SB // Dh):
                psum = psum + p[:, i * Dh:(i + 1) * Dh]
            l_new = alpha * l_old + psum
            pb = p.astype(jnp.bfloat16)
            wait_kv(slot, 1)
            pv = None
            for j in range(HG):
                oj = jnp.dot(pb, v_buf[slot, j], preferred_element_type=jnp.float32)
                pv = oj if pv is None else jnp.where(row_o == j, oj, pv)
            acc_new = alpha * acc_old + pv

            @pl.when(c == last)
            def _():
                o_scr[br, pl.ds(grow, HG), :] = acc_new / jnp.sum(l_new, axis=-1, keepdims=True)
            carry = (m_new, l_new, acc_new)
        else:
            wait_kv(slot, 0); wait_kv(slot, 1)

        t2 = t + NBUF
        @pl.when(jnp.logical_and(t2 >= offA, t2 < offA + nA))
        def _():
            issue_A(t2, slot)
        @pl.when(jnp.logical_and(t2 >= offB, t2 < offB + nB))
        def _():
            issue_B(t2, slot)
        for i in range(NBUF - 1):
            @pl.when(t2 == n + i)
            def _():
                for u in range(wo_per):
                    issue_wo(i * wo_per + u)
        return carry

    z = jnp.zeros((HG, Dh), jnp.float32)
    lax.fori_loop(0, n, body, (z, z, z))

    for c in range((NBUF - 1) * wo_per, NWO):
        issue_wo(c)
    if compute:
        for a in range(2):
            if hoffs[a]:
                o_scr[a, HG - hoffs[a]:HG, :] = o_scr[a, NH + HG - hoffs[a]:NH + HG, :]
    y = [None, None]
    hi = cfg['woprio']; lo = 1 - hi
    lead = cfg['lead']
    order = [(hi, c) for c in range(min(lead, NWO))]
    for c in range(NWO):
        if c + lead < NWO: order.append((hi, c + lead))
        order.append((lo, c))
    for (a, c) in order:
        parts = wo_parts(c, a)
        for part in parts:
            g0, gw, _ = part
            if not compute:
                wait_wo(c, part, a); continue
            lhs = jnp.concatenate(
                [o_scr[a, pl.ds(gq * NWO + c + HG - hoffs[a], B, stride=H), :] for gq in range(g0, g0 + gw)],
                axis=-1).astype(jnp.bfloat16)
            wait_wo(c, part, a)
            w = wo_buf[a, pl.ds(g0, gw), pl.ds(c * Dh, Dh), :].reshape(gw * Dh, D)
            part_y = jnp.dot(lhs, w, preferred_element_type=jnp.float32)
            y[a] = part_y if y[a] is None else y[a] + part_y
            if c == NWO - 1 and part == parts[-1]:
                o_ref[:, a * D:(a + 1) * D] = y[a].astype(o_ref.dtype)
    if not compute:
        o_ref[...] = jnp.zeros_like(o_ref)


def build(**kw):
    cfg = dict(DEFAULT); cfg.update(kw)
    @jax.jit
    def fn(A_x, A_k_cache, A_v_cache, A_wq, A_wo, B_x, B_k_cache, B_v_cache, B_wq, B_wo):
        B, Sq, D = A_x.shape
        _, H, S, Dh = A_k_cache.shape
        W = min(4096, max(256, S // 4))
        scale = Dh ** -0.5
        HD = H * Dh
        SB, NBUF = cfg['SB'], cfg['NBUF']
        any_spec = pl.BlockSpec(memory_space=pl.ANY)
        kv = lambda t: t.reshape(B * H, S, Dh)
        wq = lambda t: t.reshape(WQG, D // WQG, HD)
        wo = lambda t: t.reshape(WOG, HD // WOG, D)
        out = pl.pallas_call(
            functools.partial(_kernel, scale=scale, B=B, H=H, S=S, W=W, D=D, Dh=Dh, cfg=cfg),
            in_specs=[any_spec] * 10,
            out_specs=pl.BlockSpec(memory_space=pltpu.VMEM),
            out_shape=jax.ShapeDtypeStruct((B, 2 * D), A_x.dtype),
            scratch_shapes=[
                pltpu.VMEM((2, B, D), jnp.bfloat16),
                pltpu.VMEM((2, WQG, D // WQG, HD), jnp.bfloat16),
                pltpu.VMEM((2, WOG, HD // WOG, D), jnp.bfloat16),
                pltpu.VMEM((NBUF, HG, SB, Dh), jnp.bfloat16),
                pltpu.VMEM((NBUF, HG, SB, Dh), jnp.bfloat16),
                pltpu.VMEM((2, B * H + HG, Dh), jnp.float32),
                pltpu.VMEM((2, B * H + HG, Dh), jnp.float32),
            ],
            compiler_params=pltpu.CompilerParams(vmem_limit_bytes=64 * 1024 * 1024, disable_bounds_checks=cfg['dbc']),
        )(A_x.reshape(B, D), B_x.reshape(B, D), wq(A_wq), wq(B_wq), wo(A_wo), wo(B_wo),
          kv(A_k_cache), kv(A_v_cache), kv(B_k_cache), kv(B_v_cache))
        return out.reshape(B, Sq, 2 * D)
    return fn

pallas_concat_heads__sliding_block_cached__mha_block_cached__decode_kernel = build()
```

```python
import functools

import jax
import jax.numpy as jnp
from jax import lax
import jax.experimental.pallas as pl
import jax.experimental.pallas.tpu as pltpu

_NT = (((1,), (1,)), ((), ()))

HG = 8
SB = 512
CR = 16
NBUF = 3
WQG = 5
WQC = 256
QC = 1024
WOG = 4
WO_PER_STEP = 2
HOFF = (2, 4)
N_SEM_FIXED = 4


def _body(ax_hbm, bx_hbm, awq_hbm, bwq_hbm, awo_hbm, bwo_hbm,
          ak_hbm, av_hbm, bk_hbm, bv_hbm, o_ref,
          x_buf, wq_buf, wo_buf, k_buf, v_buf, q_scr, o_scr, sems,
          *, scale, B, H, S, W, D, Dh):
    NH = B * H
    G = NH // HG
    ncA, ncB = W // SB, S // SB
    nA, nB = G * ncA, G * ncB
    n = nA + nB
    HD = H * Dh
    NWO = wo_buf.shape[2] // Dh

    x_sem = lambda a: sems.at[a]
    wq_sem = lambda a: sems.at[2 + a]
    kv_sem = lambda slot, a: sems.at[N_SEM_FIXED + 2 * slot + a]
    wo_sem = lambda i, a: sems.at[N_SEM_FIXED + 2 * NBUF + 2 * i + a]

    def wait_all(dst, sem):
        pltpu.make_async_copy(dst, dst, sem).wait()

    def issue_wq():
        for r0 in range(0, wq_buf.shape[2], 8):
            for c0 in range(0, HD, WQC):
                for a, src in enumerate((awq_hbm, bwq_hbm)):
                    pltpu.make_async_copy(
                        src.at[:, pl.ds(r0, 8), pl.ds(c0, WQC)],
                        wq_buf.at[a, :, pl.ds(r0, 8), pl.ds(c0, WQC)],
                        wq_sem(a)).start(priority=a)

    def wo_parts(c, a):
        if c < NWO - 1 or a == 0:
            return [(0, WOG, c)]
        return [(i, 1, NWO - 1 + i) for i in range(WOG)]

    def issue_wo(c):
        lists = []
        for a, src in enumerate((awo_hbm, bwo_hbm)):
            lst = []
            for g0, gw, si in wo_parts(c, a):
                pr = 8 * (WOG // gw)
                for r0 in range(c * Dh, (c + 1) * Dh, pr):
                    lst.append(pltpu.make_async_copy(
                        src.at[pl.ds(g0, gw), pl.ds(r0, pr)],
                        wo_buf.at[a, pl.ds(g0, gw), pl.ds(r0, pr)],
                        wo_sem(si, a)))
            lists.append(lst)
        for da, db in zip(*lists):
            da.start(priority=0)
            db.start(priority=1)

    def issue_kv_parts(k_hbm, v_hbm, parts, s0, slot):
        for j in range(SB // CR):
            for a, src, buf in ((0, k_hbm, k_buf), (1, v_hbm, v_buf)):
                for h0, hn, d0 in parts:
                    pltpu.make_async_copy(
                        src.at[pl.ds(h0, hn), pl.ds(s0 + j * CR, CR)],
                        buf.at[slot, pl.ds(d0, hn), pl.ds(j * CR, CR)],
                        kv_sem(slot, a)).start(priority=1 - a)

    def issue_kv(k_hbm, v_hbm, g, s0, slot, hoff):
        def plain():
            issue_kv_parts(k_hbm, v_hbm, [(g * HG + hoff, HG, 0)], s0, slot)

        def wrap():
            issue_kv_parts(
                k_hbm, v_hbm,
                [(NH - (HG - hoff), HG - hoff, 0), (0, hoff, HG - hoff)],
                s0, slot)

        if isinstance(g, int):
            wrap() if g == G - 1 else plain()
        else:
            pl.when(g < G - 1)(plain)
            pl.when(g == G - 1)(wrap)

    def issue_a(t, slot):
        issue_kv(ak_hbm, av_hbm, t // ncA, (S - W) + (t % ncA) * SB, slot, HOFF[0])

    def issue_b(t, slot):
        tb = t - nA
        issue_kv(bk_hbm, bv_hbm, tb // ncB, (tb % ncB) * SB, slot, HOFF[1])

    def q_proj(a):
        wait_all(wq_buf.at[a], wq_sem(a))
        base = HG - HOFF[a]
        for c in range(HD // QC):
            w = wq_buf[a, :, :, pl.ds(c * QC, QC)].reshape(D, QC)
            q = jnp.dot(x_buf[a], w, preferred_element_type=jnp.float32)
            for j in range(QC // Dh):
                h = c * (QC // Dh) + j
                qh = q[:, j * Dh:(j + 1) * Dh]
                q_scr[a, pl.ds(base + h, B, stride=H), :] = qh
                if h < HOFF[a]:
                    q_scr[a, pl.ds(NH + base + h, 1), :] = qh[0:1]

    xa = pltpu.make_async_copy(ax_hbm, x_buf.at[0], x_sem(0))
    xb = pltpu.make_async_copy(bx_hbm, x_buf.at[1], x_sem(1))
    xa.start(priority=0)
    xb.start(priority=1)
    issue_wq()
    for t in range(NBUF - 1):
        issue_a(t, t)
    xa.wait()
    xb.wait()
    q_proj(0)
    issue_a(NBUF - 1, NBUF - 1)
    q_proj(1)

    row_s = lax.broadcasted_iota(jnp.int32, (HG, SB), 0)
    row_o = lax.broadcasted_iota(jnp.int32, (HG, Dh), 0)

    def step(t, carry):
        m_old, l_old, acc_old = carry
        slot = lax.rem(t, NBUF)
        is_a = t < nA
        tb = t - nA
        br = jnp.where(is_a, 0, 1)
        g = jnp.where(is_a, t // ncA, tb // ncB)
        c = jnp.where(is_a, t % ncA, tb % ncB)
        last = jnp.where(is_a, ncA - 1, ncB - 1)
        first = c == 0
        grow = pl.multiple_of((g + 1) * HG, HG)

        q8 = q_scr[br, pl.ds(grow, HG), :].astype(jnp.bfloat16)
        wait_all(k_buf.at[slot], kv_sem(slot, 0))
        s = None
        for j in range(HG):
            sj = lax.dot_general(q8, k_buf[slot, j], _NT,
                                 preferred_element_type=jnp.float32)
            s = sj if s is None else jnp.where(row_s == j, sj, s)
        s = s * scale

        m_old = jnp.where(first, -jnp.inf, m_old)
        l_old = jnp.where(first, 0.0, l_old)
        acc_old = jnp.where(first, 0.0, acc_old)
        m_new = jnp.maximum(m_old, jnp.max(s, axis=-1, keepdims=True))
        alpha = jnp.exp(m_old - m_new)
        p = jnp.exp(s - m_new[:, 0:1])
        psum = p[:, 0:Dh]
        for i in range(1, SB // Dh):
            psum = psum + p[:, i * Dh:(i + 1) * Dh]
        l_new = alpha * l_old + psum
        pb = p.astype(jnp.bfloat16)

        wait_all(v_buf.at[slot], kv_sem(slot, 1))
        pv = None
        for j in range(HG):
            oj = jnp.dot(pb, v_buf[slot, j], preferred_element_type=jnp.float32)
            pv = oj if pv is None else jnp.where(row_o == j, oj, pv)
        acc_new = alpha * acc_old + pv

        @pl.when(c == last)
        def _():
            o_scr[br, pl.ds(grow, HG), :] = (
                acc_new / jnp.sum(l_new, axis=-1, keepdims=True))

        t2 = t + NBUF

        @pl.when(t2 < nA)
        def _():
            issue_a(t2, slot)

        @pl.when(jnp.logical_and(t2 >= nA, t2 < n))
        def _():
            issue_b(t2, slot)

        for i in range(NBUF - 1):
            @pl.when(t2 == n + i)
            def _():
                for u in range(WO_PER_STEP):
                    issue_wo(i * WO_PER_STEP + u)

        return m_new, l_new, acc_new

    zero = jnp.zeros((HG, Dh), jnp.float32)
    lax.fori_loop(0, n, step, (zero, zero, zero))

    for c in range((NBUF - 1) * WO_PER_STEP, NWO):
        issue_wo(c)
    for a in range(2):
        base = HG - HOFF[a]
        o_scr[a, base:HG, :] = o_scr[a, NH + base:NH + HG, :]

    order = [(0, 0)]
    for c in range(NWO):
        if c + 1 < NWO:
            order.append((0, c + 1))
        order.append((1, c))
    y = [None, None]
    for a, c in order:
        base = HG - HOFF[a]
        for g0, gw, si in wo_parts(c, a):
            lhs = jnp.concatenate(
                [o_scr[a, pl.ds(base + gq * NWO + c, B, stride=H), :]
                 for gq in range(g0, g0 + gw)], axis=-1).astype(jnp.bfloat16)
            wait_all(wo_buf.at[a, pl.ds(g0, gw), pl.ds(c * Dh, Dh)], wo_sem(si, a))
            w = wo_buf[a, pl.ds(g0, gw), pl.ds(c * Dh, Dh), :].reshape(gw * Dh, D)
            part = jnp.dot(lhs, w, preferred_element_type=jnp.float32)
            y[a] = part if y[a] is None else y[a] + part
        if c == NWO - 1:
            o_ref[:, a * D:(a + 1) * D] = y[a].astype(o_ref.dtype)


def _kernel(*refs, n_sem, **kw):
    pl.run_scoped(lambda sems: _body(*refs, sems, **kw),
                  pltpu.SemaphoreType.DMA((n_sem,)))


@jax.jit
def pallas_concat_heads__sliding_block_cached__mha_block_cached__decode_kernel(
    A_x: jax.Array,
    A_k_cache: jax.Array,
    A_v_cache: jax.Array,
    A_wq: jax.Array,
    A_wo: jax.Array,
    B_x: jax.Array,
    B_k_cache: jax.Array,
    B_v_cache: jax.Array,
    B_wq: jax.Array,
    B_wo: jax.Array,
):
    B, Sq, D = A_x.shape
    _, H, S, Dh = A_k_cache.shape
    W = min(4096, max(256, S // 4))
    HD = H * Dh
    assert Sq == 1 and B_x.shape == A_x.shape and B_k_cache.shape == A_k_cache.shape
    assert A_wq.shape == (D, HD) and A_wo.shape == (HD, D)
    assert W % SB == 0 and S % SB == 0 and (B * H) % HG == 0
    assert (B * H // HG) * (W // SB) >= NBUF
    n_wo = HD // WOG // Dh
    n_sem = N_SEM_FIXED + 2 * NBUF + 2 * (n_wo - 1 + WOG)
    dt = A_x.dtype

    kv = lambda t: t.reshape(B * H, S, Dh)
    wq = lambda t: t.reshape(WQG, D // WQG, HD)
    wo = lambda t: t.reshape(WOG, HD // WOG, D)
    out = pl.pallas_call(
        functools.partial(_kernel, n_sem=n_sem, scale=Dh ** -0.5,
                          B=B, H=H, S=S, W=W, D=D, Dh=Dh),
        in_specs=[pl.BlockSpec(memory_space=pl.ANY)] * 10,
        out_specs=pl.BlockSpec(memory_space=pltpu.VMEM),
        out_shape=jax.ShapeDtypeStruct((B, 2 * D), dt),
        scratch_shapes=[
            pltpu.VMEM((2, B, D), dt),
            pltpu.VMEM((2, WQG, D // WQG, HD), dt),
            pltpu.VMEM((2, WOG, HD // WOG, D), dt),
            pltpu.VMEM((NBUF, HG, SB, Dh), dt),
            pltpu.VMEM((NBUF, HG, SB, Dh), dt),
            pltpu.VMEM((2, B * H + HG, Dh), jnp.float32),
            pltpu.VMEM((2, B * H + HG, Dh), jnp.float32),
        ],
        compiler_params=pltpu.CompilerParams(vmem_limit_bytes=64 * 1024 * 1024),
    )(A_x.reshape(B, D), B_x.reshape(B, D), wq(A_wq), wq(B_wq), wo(A_wo), wo(B_wo),
      kv(A_k_cache), kv(A_v_cache), kv(B_k_cache), kv(B_v_cache))
    return out.reshape(B, Sq, 2 * D)
```

```python
import functools

import jax
import jax.numpy as jnp
from jax import lax
import jax.experimental.pallas as pl
import jax.experimental.pallas.tpu as pltpu

_NT = (((1,), (1,)), ((), ()))

HG = 8
SB = 512
CR = 16
NBUF = 3
WQG = 5
WQC = 256
QC = 1024
WOG = 4
WO_PER_STEP = 2
HOFF = (2, 4)
N_SEM_FIXED = 4


def _body(ax_hbm, bx_hbm, awq_hbm, bwq_hbm, awo_hbm, bwo_hbm,
          ak_hbm, av_hbm, bk_hbm, bv_hbm, o_ref,
          x_buf, wq_buf, wo_buf, k_buf, v_buf, q_scr, o_scr, sems,
          *, scale, B, H, S, W, D, Dh):
    NH = B * H
    G = NH // HG
    ncA, ncB = W // SB, S // SB
    nA, nB = G * ncA, G * ncB
    n = nA + nB
    HD = H * Dh
    NWO = wo_buf.shape[2] // Dh

    x_sem = lambda a: sems.at[a]
    wq_sem = lambda a: sems.at[2 + a]
    kv_sem = lambda slot, a: sems.at[N_SEM_FIXED + 2 * slot + a]
    wo_sem = lambda i, a: sems.at[N_SEM_FIXED + 2 * NBUF + 2 * i + a]

    def wait_all(dst, sem):
        pltpu.make_async_copy(dst, dst, sem).wait()

    def issue_wq():
        for r0 in range(0, wq_buf.shape[2], 8):
            for c0 in range(0, HD, WQC):
                for a, src in enumerate((awq_hbm, bwq_hbm)):
                    pltpu.make_async_copy(
                        src.at[:, pl.ds(r0, 8), pl.ds(c0, WQC)],
                        wq_buf.at[a, :, pl.ds(r0, 8), pl.ds(c0, WQC)],
                        wq_sem(a)).start(priority=a)

    def wo_parts(c, a):
        if c < NWO - 1 or a == 0:
            return [(0, WOG, c)]
        return [(i, 1, NWO - 1 + i) for i in range(WOG)]

    def issue_wo(c):
        lists = []
        for a, src in enumerate((awo_hbm, bwo_hbm)):
            lst = []
            for g0, gw, si in wo_parts(c, a):
                pr = 8 * (WOG // gw)
                for r0 in range(c * Dh, (c + 1) * Dh, pr):
                    lst.append(pltpu.make_async_copy(
                        src.at[pl.ds(g0, gw), pl.ds(r0, pr)],
                        wo_buf.at[a, pl.ds(g0, gw), pl.ds(r0, pr)],
                        wo_sem(si, a)))
            lists.append(lst)
        for da, db in zip(*lists):
            da.start(priority=0)
            db.start(priority=1)

    def issue_kv_parts(k_hbm, v_hbm, parts, s0, slot):
        srcs, bufs = (k_hbm, v_hbm), (k_buf, v_buf)
        for j in range(SB // CR):
            for p in range(2):
                for i, (h0, hn, d0) in enumerate(parts):
                    a = (p + i) % 2
                    pltpu.make_async_copy(
                        srcs[a].at[pl.ds(h0, hn), pl.ds(s0 + j * CR, CR)],
                        bufs[a].at[slot, pl.ds(d0, hn), pl.ds(j * CR, CR)],
                        kv_sem(slot, a)).start(priority=1 - p)

    def issue_kv(k_hbm, v_hbm, g, s0, slot, hoff):
        def plain():
            issue_kv_parts(k_hbm, v_hbm, [(g * HG + hoff, HG, 0)], s0, slot)

        def wrap():
            issue_kv_parts(
                k_hbm, v_hbm,
                [(NH - (HG - hoff), HG - hoff, 0), (0, hoff, HG - hoff)],
                s0, slot)

        if isinstance(g, int):
            wrap() if g == G - 1 else plain()
        else:
            pl.when(g < G - 1)(plain)
            pl.when(g == G - 1)(wrap)

    def issue_a(t, slot):
        issue_kv(ak_hbm, av_hbm, t // ncA, (S - W) + (t % ncA) * SB, slot, HOFF[0])

    def issue_b(t, slot):
        tb = t - nA
        issue_kv(bk_hbm, bv_hbm, tb // ncB, (tb % ncB) * SB, slot, HOFF[1])

    def q_proj(a):
        wait_all(wq_buf.at[a], wq_sem(a))
        base = HG - HOFF[a]
        for c in range(HD // QC):
            w = wq_buf[a, :, :, pl.ds(c * QC, QC)].reshape(D, QC)
            q = jnp.dot(x_buf[a], w, preferred_element_type=jnp.float32)
            for j in range(QC // Dh):
                h = c * (QC // Dh) + j
                qh = q[:, j * Dh:(j + 1) * Dh]
                q_scr[a, pl.ds(base + h, B, stride=H), :] = qh
                if h < HOFF[a]:
                    q_scr[a, pl.ds(NH + base + h, 1), :] = qh[0:1]

    xa = pltpu.make_async_copy(ax_hbm, x_buf.at[0], x_sem(0))
    xb = pltpu.make_async_copy(bx_hbm, x_buf.at[1], x_sem(1))
    xa.start(priority=0)
    xb.start(priority=1)
    issue_wq()
    for t in range(NBUF - 1):
        issue_a(t, t)
    xa.wait()
    xb.wait()
    q_proj(0)
    issue_a(NBUF - 1, NBUF - 1)
    q_proj(1)

    row_s = lax.broadcasted_iota(jnp.int32, (HG, SB), 0)
    row_o = lax.broadcasted_iota(jnp.int32, (HG, Dh), 0)

    def step(t, carry):
        m_old, l_old, acc_old = carry
        slot = lax.rem(t, NBUF)
        is_a = t < nA
        tb = t - nA
        br = jnp.where(is_a, 0, 1)
        g = jnp.where(is_a, t // ncA, tb // ncB)
        c = jnp.where(is_a, t % ncA, tb % ncB)
        last = jnp.where(is_a, ncA - 1, ncB - 1)
        first = c == 0
        grow = pl.multiple_of((g + 1) * HG, HG)

        q8 = q_scr[br, pl.ds(grow, HG), :].astype(jnp.bfloat16)
        wait_all(k_buf.at[slot], kv_sem(slot, 0))
        s = None
        for j in range(HG):
            sj = lax.dot_general(q8, k_buf[slot, j], _NT,
                                 preferred_element_type=jnp.float32)
            s = sj if s is None else jnp.where(row_s == j, sj, s)
        s = s * scale

        m_old = jnp.where(first, -jnp.inf, m_old)
        l_old = jnp.where(first, 0.0, l_old)
        acc_old = jnp.where(first, 0.0, acc_old)
        m_new = jnp.maximum(m_old, jnp.max(s, axis=-1, keepdims=True))
        alpha = jnp.exp(m_old - m_new)
        p = jnp.exp(s - m_new[:, 0:1])
        psum = p[:, 0:Dh]
        for i in range(1, SB // Dh):
            psum = psum + p[:, i * Dh:(i + 1) * Dh]
        l_new = alpha * l_old + psum
        pb = p.astype(jnp.bfloat16)

        wait_all(v_buf.at[slot], kv_sem(slot, 1))
        pv = None
        for j in range(HG):
            oj = jnp.dot(pb, v_buf[slot, j], preferred_element_type=jnp.float32)
            pv = oj if pv is None else jnp.where(row_o == j, oj, pv)
        acc_new = alpha * acc_old + pv

        @pl.when(c == last)
        def _():
            o_scr[br, pl.ds(grow, HG), :] = (
                acc_new / jnp.sum(l_new, axis=-1, keepdims=True))

        t2 = t + NBUF

        @pl.when(t2 < nA)
        def _():
            issue_a(t2, slot)

        @pl.when(jnp.logical_and(t2 >= nA, t2 < n))
        def _():
            issue_b(t2, slot)

        for i in range(NBUF - 1):
            @pl.when(t2 == n + i)
            def _():
                for u in range(WO_PER_STEP):
                    issue_wo(i * WO_PER_STEP + u)

        return m_new, l_new, acc_new

    zero = jnp.zeros((HG, Dh), jnp.float32)
    lax.fori_loop(0, n, step, (zero, zero, zero))

    for c in range((NBUF - 1) * WO_PER_STEP, NWO):
        issue_wo(c)
    for a in range(2):
        base = HG - HOFF[a]
        o_scr[a, base:HG, :] = o_scr[a, NH + base:NH + HG, :]

    order = [(0, 0)]
    for c in range(NWO):
        if c + 1 < NWO:
            order.append((0, c + 1))
        order.append((1, c))
    y = [None, None]
    for a, c in order:
        base = HG - HOFF[a]
        for g0, gw, si in wo_parts(c, a):
            lhs = jnp.concatenate(
                [o_scr[a, pl.ds(base + gq * NWO + c, B, stride=H), :]
                 for gq in range(g0, g0 + gw)], axis=-1).astype(jnp.bfloat16)
            wait_all(wo_buf.at[a, pl.ds(g0, gw), pl.ds(c * Dh, Dh)], wo_sem(si, a))
            w = wo_buf[a, pl.ds(g0, gw), pl.ds(c * Dh, Dh), :].reshape(gw * Dh, D)
            part = jnp.dot(lhs, w, preferred_element_type=jnp.float32)
            y[a] = part if y[a] is None else y[a] + part
        if c == NWO - 1:
            o_ref[:, a * D:(a + 1) * D] = y[a].astype(o_ref.dtype)


def _kernel(*refs, n_sem, **kw):
    pl.run_scoped(lambda sems: _body(*refs, sems, **kw),
                  pltpu.SemaphoreType.DMA((n_sem,)))


@jax.jit
def pallas_concat_heads__sliding_block_cached__mha_block_cached__decode_kernel(
    A_x: jax.Array,
    A_k_cache: jax.Array,
    A_v_cache: jax.Array,
    A_wq: jax.Array,
    A_wo: jax.Array,
    B_x: jax.Array,
    B_k_cache: jax.Array,
    B_v_cache: jax.Array,
    B_wq: jax.Array,
    B_wo: jax.Array,
):
    B, Sq, D = A_x.shape
    _, H, S, Dh = A_k_cache.shape
    W = min(4096, max(256, S // 4))
    HD = H * Dh
    assert Sq == 1 and B_x.shape == A_x.shape and B_k_cache.shape == A_k_cache.shape
    assert A_wq.shape == (D, HD) and A_wo.shape == (HD, D)
    assert W % SB == 0 and S % SB == 0 and (B * H) % HG == 0
    assert (B * H // HG) * (W // SB) >= NBUF
    n_wo = HD // WOG // Dh
    n_sem = N_SEM_FIXED + 2 * NBUF + 2 * (n_wo - 1 + WOG)
    dt = A_x.dtype

    kv = lambda t: t.reshape(B * H, S, Dh)
    wq = lambda t: t.reshape(WQG, D // WQG, HD)
    wo = lambda t: t.reshape(WOG, HD // WOG, D)
    out = pl.pallas_call(
        functools.partial(_kernel, n_sem=n_sem, scale=Dh ** -0.5,
                          B=B, H=H, S=S, W=W, D=D, Dh=Dh),
        in_specs=[pl.BlockSpec(memory_space=pl.ANY)] * 10,
        out_specs=pl.BlockSpec(memory_space=pltpu.VMEM),
        out_shape=jax.ShapeDtypeStruct((B, 2 * D), dt),
        scratch_shapes=[
            pltpu.VMEM((2, B, D), dt),
            pltpu.VMEM((2, WQG, D // WQG, HD), dt),
            pltpu.VMEM((2, WOG, HD // WOG, D), dt),
            pltpu.VMEM((NBUF, HG, SB, Dh), dt),
            pltpu.VMEM((NBUF, HG, SB, Dh), dt),
            pltpu.VMEM((2, B * H + HG, Dh), jnp.float32),
            pltpu.VMEM((2, B * H + HG, Dh), jnp.float32),
        ],
        compiler_params=pltpu.CompilerParams(vmem_limit_bytes=64 * 1024 * 1024),
    )(A_x.reshape(B, D), B_x.reshape(B, D), wq(A_wq), wq(B_wq), wo(A_wo), wo(B_wo),
      kv(A_k_cache), kv(A_v_cache), kv(B_k_cache), kv(B_v_cache))
    return out.reshape(B, Sq, 2 * D)
```

```python
import functools

import jax
import jax.numpy as jnp
from jax import lax
import jax.experimental.pallas as pl
import jax.experimental.pallas.tpu as pltpu

_NT = (((1,), (1,)), ((), ()))

HG = 8
SB = 512
CR = 16
NBUF = 3
WQG = 5
WQC = 256
QC = 1024
WOG = 4
WO_PER_STEP = 2
WO_LATE = 2
PREFILL = 28
HOFF = (2, 4)
N_SEM_FIXED = 4


def _body(ax_hbm, bx_hbm, awq_hbm, bwq_hbm, awo_hbm, bwo_hbm,
          ak_hbm, av_hbm, bk_hbm, bv_hbm, o_ref,
          x_buf, wq_buf, wo_buf, k_buf, v_buf, q_scr, o_scr, sems,
          *, scale, B, H, S, W, D, Dh):
    NH = B * H
    G = NH // HG
    ncA, ncB = W // SB, S // SB
    nA, nB = G * ncA, G * ncB
    n = nA + nB
    HD = H * Dh
    NWO = wo_buf.shape[2] // Dh

    x_sem = lambda a: sems.at[a]
    wq_sem = lambda a: sems.at[2 + a]
    kv_sem = lambda slot, a: sems.at[N_SEM_FIXED + 2 * slot + a]
    wo_sem = lambda i, a: sems.at[N_SEM_FIXED + 2 * NBUF + 2 * i + a]

    def wait_all(dst, sem):
        pltpu.make_async_copy(dst, dst, sem).wait()

    def issue_wq():
        i = 0
        for r0 in range(0, wq_buf.shape[2], 8):
            for c0 in range(0, HD, WQC):
                for a, src in enumerate((awq_hbm, bwq_hbm)):
                    prio = 1 if i < PREFILL else (i - PREFILL) % 2
                    pltpu.make_async_copy(
                        src.at[:, pl.ds(r0, 8), pl.ds(c0, WQC)],
                        wq_buf.at[a, :, pl.ds(r0, 8), pl.ds(c0, WQC)],
                        wq_sem(a)).start(priority=prio)
                    i += 1

    def wo_parts(c, a):
        if c < NWO - 1 or a == 0:
            return [(0, WOG, c)]
        return [(i, 1, NWO - 1 + i) for i in range(WOG)]

    def issue_wo(c):
        lists = []
        for a, src in enumerate((awo_hbm, bwo_hbm)):
            lst = []
            for g0, gw, si in wo_parts(c, a):
                pr = 8 * (WOG // gw)
                for r0 in range(c * Dh, (c + 1) * Dh, pr):
                    lst.append(pltpu.make_async_copy(
                        src.at[pl.ds(g0, gw), pl.ds(r0, pr)],
                        wo_buf.at[a, pl.ds(g0, gw), pl.ds(r0, pr)],
                        wo_sem(si, a)))
            lists.append(lst)
        for da, db in zip(*lists):
            da.start(priority=0)
            db.start(priority=1)

    def issue_kv_parts(k_hbm, v_hbm, parts, s0, slot):
        srcs, bufs = (k_hbm, v_hbm), (k_buf, v_buf)
        for j in range(SB // CR):
            for p in range(2):
                for i, (h0, hn, d0) in enumerate(parts):
                    a = (p + i) % 2
                    pltpu.make_async_copy(
                        srcs[a].at[pl.ds(h0, hn), pl.ds(s0 + j * CR, CR)],
                        bufs[a].at[slot, pl.ds(d0, hn), pl.ds(j * CR, CR)],
                        kv_sem(slot, a)).start(priority=1 - p)

    def issue_kv(k_hbm, v_hbm, g, s0, slot, hoff):
        def plain():
            issue_kv_parts(k_hbm, v_hbm, [(g * HG + hoff, HG, 0)], s0, slot)

        def wrap():
            issue_kv_parts(
                k_hbm, v_hbm,
                [(NH - (HG - hoff), HG - hoff, 0), (0, hoff, HG - hoff)],
                s0, slot)

        if isinstance(g, int):
            wrap() if g == G - 1 else plain()
        else:
            pl.when(g < G - 1)(plain)
            pl.when(g == G - 1)(wrap)

    def issue_a(t, slot):
        issue_kv(ak_hbm, av_hbm, t // ncA, (S - W) + (t % ncA) * SB, slot, HOFF[0])

    def issue_b(t, slot):
        tb = t - nA
        issue_kv(bk_hbm, bv_hbm, tb // ncB, (tb % ncB) * SB, slot, HOFF[1])

    def q_proj(a):
        wait_all(wq_buf.at[a], wq_sem(a))
        base = HG - HOFF[a]
        for c in range(HD // QC):
            w = wq_buf[a, :, :, pl.ds(c * QC, QC)].reshape(D, QC)
            q = jnp.dot(x_buf[a], w, preferred_element_type=jnp.float32)
            for j in range(QC // Dh):
                h = c * (QC // Dh) + j
                qh = q[:, j * Dh:(j + 1) * Dh]
                q_scr[a, pl.ds(base + h, B, stride=H), :] = qh
                if h < HOFF[a]:
                    q_scr[a, pl.ds(NH + base + h, 1), :] = qh[0:1]

    xa = pltpu.make_async_copy(ax_hbm, x_buf.at[0], x_sem(0))
    xb = pltpu.make_async_copy(bx_hbm, x_buf.at[1], x_sem(1))
    xa.start(priority=0)
    xb.start(priority=1)
    issue_wq()
    for t in range(NBUF - 1):
        issue_a(t, t)
    xa.wait()
    xb.wait()
    q_proj(0)
    issue_a(NBUF - 1, NBUF - 1)
    q_proj(1)

    row_s = lax.broadcasted_iota(jnp.int32, (HG, SB), 0)
    row_o = lax.broadcasted_iota(jnp.int32, (HG, Dh), 0)

    def step(t, carry):
        m_old, l_old, acc_old = carry
        slot = lax.rem(t, NBUF)
        is_a = t < nA
        tb = t - nA
        br = jnp.where(is_a, 0, 1)
        g = jnp.where(is_a, t // ncA, tb // ncB)
        c = jnp.where(is_a, t % ncA, tb % ncB)
        last = jnp.where(is_a, ncA - 1, ncB - 1)
        first = c == 0
        grow = pl.multiple_of((g + 1) * HG, HG)

        q8 = q_scr[br, pl.ds(grow, HG), :].astype(jnp.bfloat16)
        wait_all(k_buf.at[slot], kv_sem(slot, 0))
        s = None
        for j in range(HG):
            sj = lax.dot_general(q8, k_buf[slot, j], _NT,
                                 preferred_element_type=jnp.float32)
            s = sj if s is None else jnp.where(row_s == j, sj, s)
        s = s * scale

        m_old = jnp.where(first, -jnp.inf, m_old)
        l_old = jnp.where(first, 0.0, l_old)
        acc_old = jnp.where(first, 0.0, acc_old)
        m_new = jnp.maximum(m_old, jnp.max(s, axis=-1, keepdims=True))
        alpha = jnp.exp(m_old - m_new)
        p = jnp.exp(s - m_new[:, 0:1])
        psum = p[:, 0:Dh]
        for i in range(1, SB // Dh):
            psum = psum + p[:, i * Dh:(i + 1) * Dh]
        l_new = alpha * l_old + psum
        pb = p.astype(jnp.bfloat16)

        wait_all(v_buf.at[slot], kv_sem(slot, 1))
        pv = None
        for j in range(HG):
            oj = jnp.dot(pb, v_buf[slot, j], preferred_element_type=jnp.float32)
            pv = oj if pv is None else jnp.where(row_o == j, oj, pv)
        acc_new = alpha * acc_old + pv

        @pl.when(c == last)
        def _():
            o_scr[br, pl.ds(grow, HG), :] = (
                acc_new / jnp.sum(l_new, axis=-1, keepdims=True))

        t2 = t + NBUF

        @pl.when(t2 < nA)
        def _():
            issue_a(t2, slot)

        @pl.when(jnp.logical_and(t2 >= nA, t2 < n))
        def _():
            issue_b(t2, slot)

        for i in range(NBUF - 1):
            @pl.when(t2 == n + i)
            def _():
                for u in range(WO_PER_STEP):
                    issue_wo(i * WO_PER_STEP + u)

        return m_new, l_new, acc_new

    zero = jnp.zeros((HG, Dh), jnp.float32)
    lax.fori_loop(0, n, step, (zero, zero, zero))

    for c in range((NBUF - 1) * WO_PER_STEP, NWO - WO_LATE):
        issue_wo(c)
    for a in range(2):
        base = HG - HOFF[a]
        o_scr[a, base:HG, :] = o_scr[a, NH + base:NH + HG, :]

    order = [(0, 0)]
    for c in range(NWO):
        if c + 1 < NWO:
            order.append((0, c + 1))
        order.append((1, c))
    y = [None, None]
    for a, c in order:
        if (a, c) == (1, 1):
            for c2 in range(NWO - WO_LATE, NWO):
                issue_wo(c2)
        base = HG - HOFF[a]
        for g0, gw, si in wo_parts(c, a):
            lhs = jnp.concatenate(
                [o_scr[a, pl.ds(base + gq * NWO + c, B, stride=H), :]
                 for gq in range(g0, g0 + gw)], axis=-1).astype(jnp.bfloat16)
            wait_all(wo_buf.at[a, pl.ds(g0, gw), pl.ds(c * Dh, Dh)], wo_sem(si, a))
            w = wo_buf[a, pl.ds(g0, gw), pl.ds(c * Dh, Dh), :].reshape(gw * Dh, D)
            part = jnp.dot(lhs, w, preferred_element_type=jnp.float32)
            y[a] = part if y[a] is None else y[a] + part
        if c == NWO - 1:
            o_ref[:, a * D:(a + 1) * D] = y[a].astype(o_ref.dtype)


def _kernel(*refs, n_sem, **kw):
    pl.run_scoped(lambda sems: _body(*refs, sems, **kw),
                  pltpu.SemaphoreType.DMA((n_sem,)))


@jax.jit
def pallas_concat_heads__sliding_block_cached__mha_block_cached__decode_kernel(
    A_x: jax.Array,
    A_k_cache: jax.Array,
    A_v_cache: jax.Array,
    A_wq: jax.Array,
    A_wo: jax.Array,
    B_x: jax.Array,
    B_k_cache: jax.Array,
    B_v_cache: jax.Array,
    B_wq: jax.Array,
    B_wo: jax.Array,
):
    B, Sq, D = A_x.shape
    _, H, S, Dh = A_k_cache.shape
    W = min(4096, max(256, S // 4))
    HD = H * Dh
    assert Sq == 1 and B_x.shape == A_x.shape and B_k_cache.shape == A_k_cache.shape
    assert A_wq.shape == (D, HD) and A_wo.shape == (HD, D)
    assert W % SB == 0 and S % SB == 0 and (B * H) % HG == 0
    assert (B * H // HG) * (W // SB) >= NBUF
    n_wo = HD // WOG // Dh
    assert n_wo - WO_LATE >= max((NBUF - 1) * WO_PER_STEP, 3)
    n_sem = N_SEM_FIXED + 2 * NBUF + 2 * (n_wo - 1 + WOG)
    dt = A_x.dtype

    kv = lambda t: t.reshape(B * H, S, Dh)
    wq = lambda t: t.reshape(WQG, D // WQG, HD)
    wo = lambda t: t.reshape(WOG, HD // WOG, D)
    out = pl.pallas_call(
        functools.partial(_kernel, n_sem=n_sem, scale=Dh ** -0.5,
                          B=B, H=H, S=S, W=W, D=D, Dh=Dh),
        in_specs=[pl.BlockSpec(memory_space=pl.ANY)] * 10,
        out_specs=pl.BlockSpec(memory_space=pltpu.VMEM),
        out_shape=jax.ShapeDtypeStruct((B, 2 * D), dt),
        scratch_shapes=[
            pltpu.VMEM((2, B, D), dt),
            pltpu.VMEM((2, WQG, D // WQG, HD), dt),
            pltpu.VMEM((2, WOG, HD // WOG, D), dt),
            pltpu.VMEM((NBUF, HG, SB, Dh), dt),
            pltpu.VMEM((NBUF, HG, SB, Dh), dt),
            pltpu.VMEM((2, B * H + HG, Dh), jnp.float32),
            pltpu.VMEM((2, B * H + HG, Dh), jnp.float32),
        ],
        compiler_params=pltpu.CompilerParams(vmem_limit_bytes=64 * 1024 * 1024),
    )(A_x.reshape(B, D), B_x.reshape(B, D), wq(A_wq), wq(B_wq), wo(A_wo), wo(B_wo),
      kv(A_k_cache), kv(A_v_cache), kv(B_k_cache), kv(B_v_cache))
    return out.reshape(B, Sq, 2 * D)
```

```python
import functools

import jax
import jax.numpy as jnp
from jax import lax
import jax.experimental.pallas as pl
import jax.experimental.pallas.tpu as pltpu

_NT = (((1,), (1,)), ((), ()))

HG = 8
SB = 512
CR = 16
NBUF = 3
WQG = 5
WQC = 256
QC = 1024
WOG = 4
WO_PER_STEP = 2
WO_LATE = 2
PREFILL = 28
HOFF = (2, 4)
N_SEM_FIXED = 4


def _body(ax_hbm, bx_hbm, awq_hbm, bwq_hbm, awo_hbm, bwo_hbm,
          ak_hbm, av_hbm, bk_hbm, bv_hbm, o_ref,
          x_buf, wq_buf, wo_buf, k_buf, v_buf, q_scr, o_scr, sems,
          *, scale, B, H, S, W, D, Dh):
    NH = B * H
    G = NH // HG
    ncA, ncB = W // SB, S // SB
    nA, nB = G * ncA, G * ncB
    n = nA + nB
    HD = H * Dh
    NWO = wo_buf.shape[2] // Dh

    x_sem = lambda a: sems.at[a]
    wq_sem = lambda a: sems.at[2 + a]
    kv_sem = lambda slot, a: sems.at[N_SEM_FIXED + 2 * slot + a]
    wo_sem = lambda i, a: sems.at[N_SEM_FIXED + 2 * NBUF + 2 * i + a]

    def wait_all(dst, sem):
        pltpu.make_async_copy(dst, dst, sem).wait()

    def issue_wq():
        i = 0
        for r in range(wq_buf.shape[2]):
            for c0 in range(0, HD, WQC):
                for a, src in enumerate((awq_hbm, bwq_hbm)):
                    prio = 1 if i < PREFILL else (i - PREFILL) % 2
                    pltpu.make_async_copy(
                        src.at[:, r, :, pl.ds(c0, WQC)],
                        wq_buf.at[a, :, r, :, pl.ds(c0, WQC)],
                        wq_sem(a)).start(priority=prio)
                    i += 1

    def wo_parts(c, a):
        if c < NWO - 1 or a == 0:
            return [(0, WOG, c)]
        return [(i, 1, NWO - 1 + i) for i in range(WOG)]

    def issue_wo(c):
        lists = []
        for a, src in enumerate((awo_hbm, bwo_hbm)):
            lst = []
            for g0, gw, si in wo_parts(c, a):
                gp = min(gw, 2)
                pr = 32 // gp
                for r0 in range(c * Dh, (c + 1) * Dh, pr):
                    for g1 in range(g0, g0 + gw, gp):
                        lst.append(pltpu.make_async_copy(
                            src.at[pl.ds(g1, gp), pl.ds(r0, pr)],
                            wo_buf.at[a, pl.ds(g1, gp), pl.ds(r0, pr)],
                            wo_sem(si, a)))
            lists.append(lst)
        for da, db in zip(*lists):
            da.start(priority=0)
            db.start(priority=1)

    def issue_kv_parts(k_hbm, v_hbm, parts, s0, slot):
        srcs, bufs = (k_hbm, v_hbm), (k_buf, v_buf)
        for j in range(SB // CR):
            for p in range(2):
                for i, (h0, hn, d0) in enumerate(parts):
                    a = (p + i) % 2
                    pltpu.make_async_copy(
                        srcs[a].at[pl.ds(h0, hn), pl.ds(s0 + j * CR, CR)],
                        bufs[a].at[slot, pl.ds(d0, hn), pl.ds(j * CR, CR)],
                        kv_sem(slot, a)).start(priority=1 - p)

    def issue_kv(k_hbm, v_hbm, g, s0, slot, hoff):
        def plain():
            issue_kv_parts(k_hbm, v_hbm, [(g * HG + hoff, HG, 0)], s0, slot)

        def wrap():
            issue_kv_parts(
                k_hbm, v_hbm,
                [(NH - (HG - hoff), HG - hoff, 0), (0, hoff, HG - hoff)],
                s0, slot)

        if isinstance(g, int):
            wrap() if g == G - 1 else plain()
        else:
            pl.when(g < G - 1)(plain)
            pl.when(g == G - 1)(wrap)

    def issue_a(t, slot):
        issue_kv(ak_hbm, av_hbm, t // ncA, (S - W) + (t % ncA) * SB, slot, HOFF[0])

    def issue_b(t, slot):
        tb = t - nA
        issue_kv(bk_hbm, bv_hbm, tb // ncB, (tb % ncB) * SB, slot, HOFF[1])

    def q_proj(a):
        wait_all(wq_buf.at[a], wq_sem(a))
        base = HG - HOFF[a]
        for c in range(HD // QC):
            w = wq_buf[a, :, :, :, pl.ds(c * QC, QC)].reshape(D, QC)
            q = jnp.dot(x_buf[a], w, preferred_element_type=jnp.float32)
            for j in range(QC // Dh):
                h = c * (QC // Dh) + j
                qh = q[:, j * Dh:(j + 1) * Dh]
                q_scr[a, pl.ds(base + h, B, stride=H), :] = qh
                if h < HOFF[a]:
                    q_scr[a, pl.ds(NH + base + h, 1), :] = qh[0:1]

    xa = pltpu.make_async_copy(ax_hbm, x_buf.at[0], x_sem(0))
    xb = pltpu.make_async_copy(bx_hbm, x_buf.at[1], x_sem(1))
    xa.start(priority=0)
    xb.start(priority=1)
    issue_wq()
    for t in range(NBUF - 1):
        issue_a(t, t)
    xa.wait()
    xb.wait()
    q_proj(0)
    issue_a(NBUF - 1, NBUF - 1)
    q_proj(1)

    row_s = lax.broadcasted_iota(jnp.int32, (HG, SB), 0)
    row_o = lax.broadcasted_iota(jnp.int32, (HG, Dh), 0)

    def step(t, carry):
        m_old, l_old, acc_old = carry
        slot = lax.rem(t, NBUF)
        is_a = t < nA
        tb = t - nA
        br = jnp.where(is_a, 0, 1)
        g = jnp.where(is_a, t // ncA, tb // ncB)
        c = jnp.where(is_a, t % ncA, tb % ncB)
        last = jnp.where(is_a, ncA - 1, ncB - 1)
        first = c == 0
        grow = pl.multiple_of((g + 1) * HG, HG)

        q8 = q_scr[br, pl.ds(grow, HG), :].astype(jnp.bfloat16)
        wait_all(k_buf.at[slot], kv_sem(slot, 0))
        s = None
        for j in range(HG):
            sj = lax.dot_general(q8, k_buf[slot, j], _NT,
                                 preferred_element_type=jnp.float32)
            s = sj if s is None else jnp.where(row_s == j, sj, s)
        s = s * scale

        m_old = jnp.where(first, -jnp.inf, m_old)
        l_old = jnp.where(first, 0.0, l_old)
        acc_old = jnp.where(first, 0.0, acc_old)
        m_new = jnp.maximum(m_old, jnp.max(s, axis=-1, keepdims=True))
        alpha = jnp.exp(m_old - m_new)
        p = jnp.exp(s - m_new[:, 0:1])
        psum = p[:, 0:Dh]
        for i in range(1, SB // Dh):
            psum = psum + p[:, i * Dh:(i + 1) * Dh]
        l_new = alpha * l_old + psum
        pb = p.astype(jnp.bfloat16)

        wait_all(v_buf.at[slot], kv_sem(slot, 1))
        pv = None
        for j in range(HG):
            oj = jnp.dot(pb, v_buf[slot, j], preferred_element_type=jnp.float32)
            pv = oj if pv is None else jnp.where(row_o == j, oj, pv)
        acc_new = alpha * acc_old + pv

        @pl.when(c == last)
        def _():
            o_scr[br, pl.ds(grow, HG), :] = (
                acc_new / jnp.sum(l_new, axis=-1, keepdims=True))

        t2 = t + NBUF

        @pl.when(t2 < nA)
        def _():
            issue_a(t2, slot)

        @pl.when(jnp.logical_and(t2 >= nA, t2 < n))
        def _():
            issue_b(t2, slot)

        for i in range(NBUF - 1):
            @pl.when(t2 == n + i)
            def _():
                for u in range(WO_PER_STEP):
                    issue_wo(i * WO_PER_STEP + u)

        return m_new, l_new, acc_new

    zero = jnp.zeros((HG, Dh), jnp.float32)
    lax.fori_loop(0, n, step, (zero, zero, zero))

    for c in range((NBUF - 1) * WO_PER_STEP, NWO - WO_LATE):
        issue_wo(c)
    for a in range(2):
        base = HG - HOFF[a]
        o_scr[a, base:HG, :] = o_scr[a, NH + base:NH + HG, :]

    order = [(0, 0)]
    for c in range(NWO):
        if c + 1 < NWO:
            order.append((0, c + 1))
        order.append((1, c))
    y = [None, None]
    for a, c in order:
        if (a, c) == (1, 1):
            for c2 in range(NWO - WO_LATE, NWO):
                issue_wo(c2)
        base = HG - HOFF[a]
        for g0, gw, si in wo_parts(c, a):
            lhs = jnp.concatenate(
                [o_scr[a, pl.ds(base + gq * NWO + c, B, stride=H), :]
                 for gq in range(g0, g0 + gw)], axis=-1).astype(jnp.bfloat16)
            wait_all(wo_buf.at[a, pl.ds(g0, gw), pl.ds(c * Dh, Dh)], wo_sem(si, a))
            w = wo_buf[a, pl.ds(g0, gw), pl.ds(c * Dh, Dh), :].reshape(gw * Dh, D)
            part = jnp.dot(lhs, w, preferred_element_type=jnp.float32)
            y[a] = part if y[a] is None else y[a] + part
        if c == NWO - 1:
            o_ref[:, a * D:(a + 1) * D] = y[a].astype(o_ref.dtype)


def _kernel(*refs, n_sem, **kw):
    pl.run_scoped(lambda sems: _body(*refs, sems, **kw),
                  pltpu.SemaphoreType.DMA((n_sem,)))


@jax.jit
def pallas_concat_heads__sliding_block_cached__mha_block_cached__decode_kernel(
    A_x: jax.Array,
    A_k_cache: jax.Array,
    A_v_cache: jax.Array,
    A_wq: jax.Array,
    A_wo: jax.Array,
    B_x: jax.Array,
    B_k_cache: jax.Array,
    B_v_cache: jax.Array,
    B_wq: jax.Array,
    B_wo: jax.Array,
):
    B, Sq, D = A_x.shape
    _, H, S, Dh = A_k_cache.shape
    W = min(4096, max(256, S // 4))
    HD = H * Dh
    assert Sq == 1 and B_x.shape == A_x.shape and B_k_cache.shape == A_k_cache.shape
    assert A_wq.shape == (D, HD) and A_wo.shape == (HD, D)
    assert W % SB == 0 and S % SB == 0 and (B * H) % HG == 0
    assert (B * H // HG) * (W // SB) >= NBUF
    n_wo = HD // WOG // Dh
    assert n_wo - WO_LATE >= max((NBUF - 1) * WO_PER_STEP, 3)
    n_sem = N_SEM_FIXED + 2 * NBUF + 2 * (n_wo - 1 + WOG)
    n_rows = B * H + H + HG
    dt = A_x.dtype

    kv = lambda t: t.reshape(B * H, S, Dh)
    wq = lambda t: t.reshape(WQG, D // WQG // 8, 8, HD)
    wo = lambda t: t.reshape(WOG, HD // WOG, D)
    out = pl.pallas_call(
        functools.partial(_kernel, n_sem=n_sem, scale=Dh ** -0.5,
                          B=B, H=H, S=S, W=W, D=D, Dh=Dh),
        in_specs=[pl.BlockSpec(memory_space=pl.ANY)] * 10,
        out_specs=pl.BlockSpec(memory_space=pltpu.VMEM),
        out_shape=jax.ShapeDtypeStruct((B, 2 * D), dt),
        scratch_shapes=[
            pltpu.VMEM((2, B, D), dt),
            pltpu.VMEM((2, WQG, D // WQG // 8, 8, HD), dt),
            pltpu.VMEM((2, WOG, HD // WOG, D), dt),
            pltpu.VMEM((NBUF, HG, SB, Dh), dt),
            pltpu.VMEM((NBUF, HG, SB, Dh), dt),
            pltpu.VMEM((2, n_rows, Dh), jnp.float32),
            pltpu.VMEM((2, n_rows, Dh), jnp.float32),
        ],
        compiler_params=pltpu.CompilerParams(vmem_limit_bytes=64 * 1024 * 1024),
    )(A_x.reshape(B, D), B_x.reshape(B, D), wq(A_wq), wq(B_wq), wo(A_wo), wo(B_wo),
      kv(A_k_cache), kv(A_v_cache), kv(B_k_cache), kv(B_v_cache))
    return out.reshape(B, Sq, 2 * D)
```
